```python
import os as _os
_os.environ.setdefault("JAX_PLATFORMS", "cpu")
import jax
import jax.numpy as jnp

def _softmax(x, axis=-1):
    return jax.nn.softmax(x, axis=axis)
def _gelu(x):
    return jax.nn.gelu(x, approximate=True)
def _silu(x):
    return jax.nn.silu(x)
def _sigmoid(x):
    return jax.nn.sigmoid(x)
def _layernorm(x, axis=-1, eps=1e-5):
    m = jnp.mean(x, axis=axis, keepdims=True)
    v = jnp.var(x, axis=axis, keepdims=True)
    return (x - m) / jnp.sqrt(v + eps)
def _scatter_add(tgt, idx, src, axis=0):
    return tgt.at[idx].add(src)
def _segment_sum(src, seg, n):
    return jax.ops.segment_sum(src, seg, n)
class _Rng:
    def __init__(self, key):
        self._k = key
    def _next(self):
        self._k, sub = jax.random.split(self._k)
        return sub
    def normal(self, shape):
        return jax.random.normal(self._next(), shape, dtype=jnp.bfloat16)
    def randint(self, lo, hi, shape):
        return jax.random.randint(self._next(), shape, lo, hi, dtype=jnp.int32)
    def uniform(self, shape, lo=0.0, hi=1.0):
        return jax.random.uniform(self._next(), shape, jnp.bfloat16, lo, hi)
    def permutation(self, n):
        return jax.random.permutation(self._next(), n)


kernel_name = 'sequential_preLN__compressed_kv_cla__dense_activation_mish__decode'

def setup_inputs():
    _rng = _Rng(jax.random.key(int.from_bytes(__import__("os").urandom(4), "little")))
    _w = (lambda a: (lambda t: t.astype(jnp.bfloat16) if jnp.issubdtype(t.dtype, jnp.floating) else t)(jnp.asarray(a)))
    def _A_setup():
        B, H, Sq, Sk, D, M = 2, 32, 1, 8192, 128, 512
        Dc = 4 * D
        return {
            "x": _w((lambda *s: _rng.normal(s) * 0.05)(B, Sq, M)),
            "c_kv": _w((lambda *s: _rng.normal(s) * 0.8)(B, Sk, Dc)),
            "w_q": _w((lambda *s: _rng.normal(s) * 0.8)(M, H, D) * (M ** -0.5)),
            "w_uk": _w((lambda *s: _rng.normal(s) * 0.8)(Dc, H, D) * (Dc ** -0.5)),
            "w_uv": _w((lambda *s: _rng.normal(s) * 0.8)(Dc, H, D) * (Dc ** -0.5)),
            "w_o": _w((lambda *s: _rng.normal(s) * 0.8)(H, D, M) * ((H * D) ** -0.5)),
        }
    _A_in = _A_setup()

    def _B_setup():
        B, S, D, F = 2, 1, 512, 1792
        return {
            "x": _w((lambda *s: _rng.normal(s) * 0.05)(B, S, D)),
            "w1": _w((lambda *s: _rng.normal(s) * 0.4)(D, F) * (D ** -0.5)),
            "b1": _w((lambda *s: _rng.normal(s) * 0.05)(F)),
            "w2": _w((lambda *s: _rng.normal(s) * 0.05)(F, D) * (F ** -0.5)),
        }
    _B_in = _B_setup()

    return {
        "A_x": _A_in["x"],
        "A_c_kv": _A_in["c_kv"],
        "A_w_q": _A_in["w_q"],
        "A_w_uk": _A_in["w_uk"],
        "A_w_uv": _A_in["w_uv"],
        "A_w_o": _A_in["w_o"],
        "B_x": _B_in["x"],
        "B_w1": _B_in["w1"],
        "B_b1": _B_in["b1"],
        "B_w2": _B_in["w2"],
    }

def reference(A_x, A_c_kv, A_w_q, A_w_uk, A_w_uv, A_w_o, B_x, B_w1, B_b1, B_w2):
    def _A_ref(x, c_kv, w_q, w_uk, w_uv, w_o):
        B, Sq, M = x.shape[0], x.shape[1], x.shape[2]
        Sk = c_kv.shape[1]
        H, D = w_q.shape[1], w_q.shape[2]
        q = jnp.einsum("bqm,mhd->bhqd", x, w_q)
        k = jnp.einsum("bkc,chd->bhkd", c_kv, w_uk)
        v = jnp.einsum("bkc,chd->bhkd", c_kv, w_uv)
        scores = jnp.einsum("bhqd,bhkd->bhqk", q, k) * (D ** -0.5)
        off = Sk - Sq
        qi = jnp.arange(Sq)[:, None]
        kj = jnp.arange(Sk)[None, :]
        cmask = kj <= (qi + off)
        scores = jnp.where(cmask[None, None], scores, -1e9)
        p = _softmax(scores, axis=-1)
        ctx = jnp.einsum("bhqk,bhkd->bhqd", p, v)
        return jnp.einsum("bhqd,hdm->bqm", ctx, w_o)

    def _B_ref(x, w1, b1, w2):
        h = jnp.einsum("bsd,df->bsf", x, w1) + b1
        sp = jnp.log1p(jnp.exp(-jnp.abs(h))) + jnp.where(h > 0, h, jnp.zeros_like(h))
        act = h * jnp.tanh(sp)
        return jnp.einsum("bsf,fd->bsd", act, w2)

    x = A_x
    h = x + _A_ref(_layernorm(x, axis=-1), A_c_kv, A_w_q, A_w_uk, A_w_uv, A_w_o)
    h2 = h + _B_ref(_layernorm(h, axis=-1), B_w1, B_b1, B_w2)
    return h2
```

```python
import functools

import jax
import jax.numpy as jnp
import jax.experimental.pallas as pl
import jax.experimental.pallas.tpu as pltpu

_B = 2
_M = 512
_H = 32
_D = 128
_C = 512
_SK = 8192
_F = 1792

_KV_CH = 2048
_KV_NCH = _SK // _KV_CH
_KV_SUB = 1024
_W2_TAIL = 256

_NT = (((1,), (1,)), ((), ()))


def _layernorm(v):
    m = jnp.mean(v, axis=-1, keepdims=True)
    c = v - m
    var = jnp.mean(c * c, axis=-1, keepdims=True)
    return c / jnp.sqrt(var + 1e-5)


def _pair_rows(w32_ref, g, jj, n):
    rows = w32_ref.shape[0]
    view = w32_ref.at[pl.ds(pl.multiple_of(4 * g, 4), rows - 12)]
    w = view[pl.ds(jj, n, stride=_H // 2), :]
    return pltpu.bitcast(w, jnp.bfloat16)


def _kernel(x_hbm, ckv_hbm, wq_hbm, wuk_hbm, wuv_hbm, wo_hbm, w1_hbm, b1_hbm, w2_hbm,
            o_ref,
            x_v, ckv_v, wq_v, wuk_v, wuv_v, wo_v, w1_v, b1_v, w2_v,
            l_s, t_s, qa_s, sems):
    f32, bf16 = jnp.float32, jnp.bfloat16

    copies = []

    def add(src, dst):
        cp = pltpu.make_async_copy(src, dst, sems.at[len(copies)])
        copies.append(cp)
        return cp

    c_wq = add(wq_hbm, wq_v)
    c_x = add(x_hbm, x_v)
    c_b1 = add(b1_hbm, b1_v)
    c_wuk = add(wuk_hbm, wuk_v)
    kv0 = len(copies)
    for b in range(_B):
        for i in range(_KV_NCH):
            add(ckv_hbm.at[b, pl.ds(i * _KV_CH, _KV_CH)], ckv_v.at[b, pl.ds(i * _KV_CH, _KV_CH)])
    c_wuv = add(wuv_hbm, wuv_v)
    c_wo = add(wo_hbm, wo_v)
    c_w1 = add(w1_hbm, w1_v)
    f0 = _F - _W2_TAIL
    c_w2a = add(w2_hbm.at[pl.ds(0, f0)], w2_v.at[pl.ds(0, f0)])
    c_w2b = add(w2_hbm.at[pl.ds(f0, _W2_TAIL)], w2_v.at[pl.ds(f0, _W2_TAIL)])
    for cp in copies:
        cp.start()

    ri = jax.lax.broadcasted_iota(jnp.int32, (128, 256), 0)
    ci = jax.lax.broadcasted_iota(jnp.int32, (128, 256), 1)
    dup = jnp.where(ri == (ci >> 1), 1.0, 0.0).astype(bf16)
    rt = jax.lax.broadcasted_iota(jnp.int32, (256, 128), 0)
    ct = jax.lax.broadcasted_iota(jnp.int32, (256, 128), 1)
    dup_t = jnp.where((rt >> 1) == ct, 1.0, 0.0).astype(bf16)

    row16 = jax.lax.broadcasted_iota(jnp.int32, (16, 2 * _C), 0)
    lane16 = jax.lax.broadcasted_iota(jnp.int32, (16, 2 * _C), 1)
    hh16 = row16 & 7
    par_ok = (lane16 & 1) == (hh16 & 1)

    def expand(v):
        return jnp.concatenate(
            [jnp.dot(v[:, 128 * t:128 * (t + 1)], dup, preferred_element_type=f32)
             for t in range(_C // 128)], axis=1)

    def store_pair_lhs(v2):
        for jj in range(4):
            keep = jnp.logical_and(par_ok, (hh16 >> 1) == jj)
            l_s[jj] = jnp.where(keep, v2, 0.0).astype(bf16)

    wq32 = wq_v.bitcast(jnp.uint32)
    wuk32 = wuk_v.bitcast(jnp.uint32)
    wuv32 = wuv_v.bitcast(jnp.uint32)

    c_x.wait()
    x2 = x_v[...].astype(f32)
    xf = jnp.concatenate(
        [jnp.broadcast_to(x2[b:b + 1], (8, _M)) for b in range(_B)], axis=0)
    xn = _layernorm(xf).astype(bf16)
    store_pair_lhs(expand(xn))

    scale = _D ** -0.5
    log2e = 1.4426950408889634

    c_wq.wait()

    def q_group(g, _):
        acc = jnp.zeros((16, _D), f32)
        for jj in range(4):
            acc = acc + jnp.dot(l_s[jj], _pair_rows(wq32, g, jj, _M),
                                preferred_element_type=f32)
        t_s[g] = acc
        return 0

    jax.lax.fori_loop(0, 4, q_group, 0)

    c_wuk.wait()
    hh_q = jax.lax.broadcasted_iota(jnp.int32, (16, _D), 0) & 7

    def qa_group(g, _):
        q = t_s[g]
        acc = jnp.zeros((16, 2 * _C), f32)
        for jj in range(4):
            lq = jnp.where((hh_q >> 1) == jj, q, 0.0).astype(bf16)
            acc = acc + jax.lax.dot_general(lq, _pair_rows(wuk32, g, jj, _C), _NT,
                                            preferred_element_type=f32)
        tm = jnp.where(par_ok, acc * (scale * log2e), 0.0).astype(bf16)
        qa = jnp.concatenate(
            [jnp.dot(tm[:, 256 * t:256 * (t + 1)], dup_t, preferred_element_type=f32)
             for t in range(_C // 128)], axis=1)
        qa_s[0, pl.ds(pl.multiple_of(8 * g, 8), 8), :] = qa[0:8]
        qa_s[1, pl.ds(pl.multiple_of(8 * g, 8), 8), :] = qa[8:16]
        return 0

    jax.lax.fori_loop(0, 4, qa_group, 0)

    for b in range(_B):
        qa = qa_s[b].astype(bf16)

        def kv_chunk(i, carry, b=b, qa=qa):
            m, l, acc = carry
            pltpu.make_async_copy(
                ckv_hbm.at[b, pl.ds(0, _KV_CH)],
                ckv_v.at[b, pl.ds(pl.multiple_of(i * _KV_CH, _KV_CH), _KV_CH)],
                sems.at[kv0 + b * _KV_NCH + i]).wait()
            for u in range(_KV_CH // _KV_SUB):
                off = pl.multiple_of(i * _KV_CH + u * _KV_SUB, _KV_SUB)
                ck = ckv_v[b, pl.ds(off, _KV_SUB), :]
                s = jax.lax.dot_general(qa, ck, _NT, preferred_element_type=f32)
                m_new = jnp.maximum(m, jnp.max(s, axis=-1, keepdims=True))
                alpha = jnp.exp2(m - m_new)
                p = jnp.exp2(s - m_new)
                l = alpha * l + jnp.sum(p, axis=-1, keepdims=True)
                acc = alpha * acc + jnp.dot(p.astype(bf16), ck, preferred_element_type=f32)
                m = m_new
            return m, l, acc

        m0 = jnp.full((_H, 1), -jnp.inf, f32)
        l0 = jnp.zeros((_H, 1), f32)
        a0 = jnp.zeros((_H, _C), f32)
        _, l, acc = jax.lax.fori_loop(0, _KV_NCH, kv_chunk, (m0, l0, a0))
        qa_s[b] = acc / l

    c_wuv.wait()

    def ctx_group(g, _):
        r0 = pl.multiple_of(8 * g, 8)
        cl = jnp.concatenate([qa_s[0, pl.ds(r0, 8), :], qa_s[1, pl.ds(r0, 8), :]], axis=0)
        cl2 = expand(cl.astype(bf16))
        acc = jnp.zeros((16, _D), f32)
        for jj in range(4):
            keep = jnp.logical_and(par_ok, (hh16 >> 1) == jj)
            lhs = jnp.where(keep, cl2, 0.0).astype(bf16)
            acc = acc + jnp.dot(lhs, _pair_rows(wuv32, g, jj, _C),
                                preferred_element_type=f32)
        t_s[g] = acc
        return 0

    jax.lax.fori_loop(0, 4, ctx_group, 0)

    c_wo.wait()

    def out_group(g, acc):
        ctx = t_s[g]
        lhs = jnp.concatenate(
            [jnp.where(hh_q == k, ctx, 0.0).astype(bf16) for k in range(8)], axis=1)
        w = wo_v[pl.ds(pl.multiple_of(g * 8 * _D, 8 * _D), 8 * _D), :]
        return acc + jnp.dot(lhs, w, preferred_element_type=f32)

    part = jax.lax.fori_loop(0, 4, out_group, jnp.zeros((16, _M), f32))
    attn = jnp.concatenate(
        [jnp.sum(part[8 * b:8 * (b + 1)], axis=0, keepdims=True) for b in range(_B)], axis=0)
    h = x2 + attn

    hn = _layernorm(h)
    hn = jnp.concatenate([hn, jnp.zeros((14, _M), f32)], axis=0).astype(bf16)
    c_b1.wait()
    c_w1.wait()
    u = jnp.dot(hn, w1_v[...], preferred_element_type=f32)[0:8]
    u = u + b1_v[...].astype(f32)[None, :]
    sp = jnp.log1p(jnp.exp(-jnp.abs(u))) + jnp.maximum(u, 0.0)
    act = u * jnp.tanh(sp)
    act = jnp.concatenate([act, jnp.zeros((8, _F), f32)], axis=0).astype(bf16)
    c_w2a.wait()
    y = jnp.dot(act[:, 0:f0], w2_v[pl.ds(0, f0), :], preferred_element_type=f32)
    c_w2b.wait()
    y = y + jnp.dot(act[:, f0:_F], w2_v[pl.ds(f0, _W2_TAIL), :], preferred_element_type=f32)
    o_ref[...] = (h + y[0:_B]).astype(o_ref.dtype)


@jax.jit
def pallas_sequential_preLN__compressed_kv_cla__dense_activation_mish__decode_kernel(
    A_x: jax.Array,
    A_c_kv: jax.Array,
    A_w_q: jax.Array,
    A_w_uk: jax.Array,
    A_w_uv: jax.Array,
    A_w_o: jax.Array,
    B_x: jax.Array,
    B_w1: jax.Array,
    B_b1: jax.Array,
    B_w2: jax.Array,
):
    del B_x
    bf16 = jnp.bfloat16
    wq = A_w_q.reshape(_M * _H, _D)
    wuk = A_w_uk.reshape(_C * _H, _D)
    wuv = A_w_uv.reshape(_C * _H, _D)
    wo = A_w_o.reshape(_H * _D, _M)
    n_dma = 4 + _B * _KV_NCH + 5
    hbm = pl.BlockSpec(memory_space=pl.ANY)
    out = pl.pallas_call(
        _kernel,
        out_shape=jax.ShapeDtypeStruct((_B, _M), A_x.dtype),
        in_specs=[hbm] * 9,
        out_specs=pl.BlockSpec(memory_space=pltpu.VMEM),
        scratch_shapes=[
            pltpu.VMEM((_B, _M), bf16),
            pltpu.VMEM((_B, _SK, _C), bf16),
            pltpu.VMEM((_M * _H, _D), bf16),
            pltpu.VMEM((_C * _H, _D), bf16),
            pltpu.VMEM((_C * _H, _D), bf16),
            pltpu.VMEM((_H * _D, _M), bf16),
            pltpu.VMEM((_M, _F), bf16),
            pltpu.VMEM((_F,), bf16),
            pltpu.VMEM((_F, _M), bf16),
            pltpu.VMEM((4, 16, 2 * _C), bf16),
            pltpu.VMEM((4, 16, _D), jnp.float32),
            pltpu.VMEM((_B, _H, _C), jnp.float32),
            pltpu.SemaphoreType.DMA((n_dma,)),
        ],
        compiler_params=pltpu.CompilerParams(vmem_limit_bytes=60 * 1024 * 1024),
    )(A_x.reshape(_B, _M), A_c_kv, wq, wuk, wuv, wo, B_w1, B_b1, B_w2)
    return out.reshape(_B, 1, _M)
```

```python
import functools

import jax
import jax.numpy as jnp
import jax.experimental.pallas as pl
import jax.experimental.pallas.tpu as pltpu

_B = 2
_M = 512
_H = 32
_D = 128
_C = 512
_SK = 8192
_F = 1792

_KV_CH = 4096
_KV_SUB = 1024
_W2_SPLITS = (896, 512, 256, 128)

_NT = (((1,), (1,)), ((), ()))


def _n_copies():
    return 7 + _B * (_SK // _KV_CH) + len(_W2_SPLITS)


def _layernorm(v):
    m = jnp.mean(v, axis=-1, keepdims=True)
    c = v - m
    var = jnp.mean(c * c, axis=-1, keepdims=True)
    return c / jnp.sqrt(var + 1e-5)


def _pair_rows(w32_ref, g, jj, n):
    rows = w32_ref.shape[0]
    view = w32_ref.at[pl.ds(pl.multiple_of(4 * g, 4), rows - 12)]
    w = view[pl.ds(jj, n, stride=_H // 2), :]
    return pltpu.bitcast(w, jnp.bfloat16)


def _body(x_hbm, ckv_hbm, wq_hbm, wuk_hbm, wuv_hbm, wo_hbm, w1_hbm, b1_hbm, w2_hbm,
          o_hbm, out_sem, out_v,
          x_v, ckv_v, wq_v, wuk_v, wuv_v, wo_v, w1_v, b1_v, w2_v,
          l_s, t_s, qa_s, cl_s, sems):
    f32, bf16 = jnp.float32, jnp.bfloat16

    n_kv = _SK // _KV_CH
    w2_off = [sum(_W2_SPLITS[:i]) for i in range(len(_W2_SPLITS))]
    copies = []

    def queue(src, dst):
        copies.append(pltpu.make_async_copy(src, dst, sems.at[len(copies)]))
        return copies[-1]

    cp_wq, cp_x, cp_b1 = queue(wq_hbm, wq_v), queue(x_hbm, x_v), queue(b1_hbm, b1_v)
    cp_wuk = queue(wuk_hbm, wuk_v)
    kv_sem0 = len(copies)
    for b in range(_B):
        for c in range(n_kv):
            sl = pl.ds(c * _KV_CH, _KV_CH)
            queue(ckv_hbm.at[b, sl], ckv_v.at[b, sl])
    cp_wuv, cp_wo, cp_w1 = queue(wuv_hbm, wuv_v), queue(wo_hbm, wo_v), queue(w1_hbm, w1_v)
    cp_w2 = [queue(w2_hbm.at[pl.ds(f0, n)], w2_v.at[pl.ds(f0, n)])
             for f0, n in zip(w2_off, _W2_SPLITS)]
    assert len(copies) == _n_copies()
    for cp in copies:
        cp.start()

    ri = jax.lax.broadcasted_iota(jnp.int32, (128, 256), 0)
    ci = jax.lax.broadcasted_iota(jnp.int32, (128, 256), 1)
    dup = jnp.where(ri == (ci >> 1), 1.0, 0.0).astype(bf16)
    rt = jax.lax.broadcasted_iota(jnp.int32, (256, 128), 0)
    ct = jax.lax.broadcasted_iota(jnp.int32, (256, 128), 1)
    dup_t = jnp.where((rt >> 1) == ct, 1.0, 0.0).astype(bf16)

    row16 = jax.lax.broadcasted_iota(jnp.int32, (16, 2 * _C), 0)
    lane16 = jax.lax.broadcasted_iota(jnp.int32, (16, 2 * _C), 1)
    hh16 = row16 & 7
    par_ok = (lane16 & 1) == (hh16 & 1)

    def expand(v):
        return jnp.concatenate(
            [jnp.dot(v[:, 128 * t:128 * (t + 1)], dup, preferred_element_type=f32)
             for t in range(_C // 128)], axis=1)

    def store_pair_lhs(v2):
        for jj in range(4):
            keep = jnp.logical_and(par_ok, (hh16 >> 1) == jj)
            l_s[jj] = jnp.where(keep, v2, 0.0).astype(bf16)

    wq32 = wq_v.bitcast(jnp.uint32)
    wuk32 = wuk_v.bitcast(jnp.uint32)
    wuv32 = wuv_v.bitcast(jnp.uint32)

    cp_x.wait()
    x2 = x_v[...].astype(f32)
    xf = jnp.concatenate(
        [jnp.broadcast_to(x2[b:b + 1], (8, _M)) for b in range(_B)], axis=0)
    xn = _layernorm(xf).astype(bf16)
    store_pair_lhs(expand(xn))
    cp_wq.wait()

    scale = _D ** -0.5
    log2e = 1.4426950408889634

    def q_group(g, _):
        acc = jnp.zeros((16, _D), f32)
        for jj in range(4):
            acc = acc + jnp.dot(l_s[jj], _pair_rows(wq32, g, jj, _M),
                                preferred_element_type=f32)
        t_s[g] = acc
        return 0

    jax.lax.fori_loop(0, 4, q_group, 0)

    cp_wuk.wait()
    hh_q = jax.lax.broadcasted_iota(jnp.int32, (16, _D), 0) & 7

    def qa_group(g, _):
        q = t_s[g]
        acc = jnp.zeros((16, 2 * _C), f32)
        for jj in range(4):
            lq = jnp.where((hh_q >> 1) == jj, q, 0.0).astype(bf16)
            acc = acc + jax.lax.dot_general(lq, _pair_rows(wuk32, g, jj, _C), _NT,
                                            preferred_element_type=f32)
        tm = jnp.where(par_ok, acc * (scale * log2e), 0.0).astype(bf16)
        qa = jnp.concatenate(
            [jnp.dot(tm[:, 256 * t:256 * (t + 1)], dup_t, preferred_element_type=f32)
             for t in range(_C // 128)], axis=1)
        qa_s[0, pl.ds(pl.multiple_of(8 * g, 8), 8), :] = qa[0:8]
        qa_s[1, pl.ds(pl.multiple_of(8 * g, 8), 8), :] = qa[8:16]
        return 0

    jax.lax.fori_loop(0, 4, qa_group, 0)

    n_sub = _SK // _KV_SUB
    sub_per_dma = _KV_CH // _KV_SUB

    def kv_step(i, carry):
        m, l, acc = carry
        b = i // n_sub
        s_idx = i - b * n_sub
        off = pl.multiple_of(s_idx * _KV_SUB, _KV_SUB)

        @pl.when(s_idx % sub_per_dma == 0)
        def _():
            sl = pl.ds(pl.multiple_of((s_idx // sub_per_dma) * _KV_CH, _KV_CH), _KV_CH)
            pltpu.make_async_copy(ckv_hbm.at[b, sl], ckv_v.at[b, sl],
                                  sems.at[kv_sem0 + i // sub_per_dma]).wait()

        first = s_idx == 0
        m = jnp.where(first, -jnp.inf, m)
        l = jnp.where(first, 0.0, l)
        acc = jnp.where(first, 0.0, acc)
        qa = qa_s[b].astype(bf16)
        ck = ckv_v[b, pl.ds(off, _KV_SUB), :]
        s = jax.lax.dot_general(qa, ck, _NT, preferred_element_type=f32)
        m_new = jnp.maximum(m, jnp.max(s, axis=-1, keepdims=True))
        alpha = jnp.exp2(m - m_new)
        p = jnp.exp2(s - m_new)
        l = alpha * l + jnp.sum(p, axis=-1, keepdims=True)
        acc = alpha * acc + jnp.dot(p.astype(bf16), ck, preferred_element_type=f32)

        @pl.when(s_idx == n_sub - 1)
        def _():
            cl_s[b] = acc / l

        return m_new, l, acc

    jax.lax.fori_loop(
        0, _B * n_sub, kv_step,
        (jnp.zeros((_H, 1), f32), jnp.zeros((_H, 1), f32), jnp.zeros((_H, _C), f32)))

    cp_wuv.wait()

    def ctx_group(g, _):
        r0 = pl.multiple_of(8 * g, 8)
        cl = jnp.concatenate([cl_s[0, pl.ds(r0, 8), :], cl_s[1, pl.ds(r0, 8), :]], axis=0)
        cl2 = expand(cl.astype(bf16))
        acc = jnp.zeros((16, _D), f32)
        for jj in range(4):
            keep = jnp.logical_and(par_ok, (hh16 >> 1) == jj)
            lhs = jnp.where(keep, cl2, 0.0).astype(bf16)
            acc = acc + jnp.dot(lhs, _pair_rows(wuv32, g, jj, _C),
                                preferred_element_type=f32)
        t_s[g] = acc
        return 0

    jax.lax.fori_loop(0, 4, ctx_group, 0)

    cp_wo.wait()

    def out_group(g, acc):
        ctx = t_s[g]
        lhs = jnp.concatenate(
            [jnp.where(hh_q == k, ctx, 0.0).astype(bf16) for k in range(8)], axis=1)
        w = wo_v[pl.ds(pl.multiple_of(g * 8 * _D, 8 * _D), 8 * _D), :]
        return acc + jnp.dot(lhs, w, preferred_element_type=f32)

    part = jax.lax.fori_loop(0, 4, out_group, jnp.zeros((16, _M), f32))
    attn = jnp.concatenate(
        [jnp.broadcast_to(jnp.sum(part[8 * b:8 * (b + 1)], axis=0, keepdims=True), (8, _M))
         for b in range(_B)], axis=0)
    h = xf + attn

    hn = _layernorm(h).astype(bf16)
    cp_b1.wait()
    cp_w1.wait()
    u = jnp.dot(hn, w1_v[...], preferred_element_type=f32)
    u = u + b1_v[...].astype(f32)[None, :]
    sp = jnp.log1p(jnp.exp(-jnp.abs(u))) + jnp.maximum(u, 0.0)
    act = (u * jnp.tanh(sp)).astype(bf16)
    y = h
    for cp, f0, n in zip(cp_w2, w2_off, _W2_SPLITS):
        cp.wait()
        y = y + jnp.dot(act[:, f0:f0 + n], w2_v[pl.ds(f0, n), :], preferred_element_type=f32)
    sub = jax.lax.broadcasted_iota(jnp.int32, (8, _M), 0)
    out_v[...] = jnp.where(sub == 0, y[0:8], y[8:16])[0:_B].astype(bf16)
    pltpu.make_async_copy(out_v, o_hbm, out_sem).start()


def _kernel(x_hbm, ckv_hbm, wq_hbm, wuk_hbm, wuv_hbm, wo_hbm, w1_hbm, b1_hbm, w2_hbm, o_hbm,
            out_sem, out_v, *scratch):
    pl.run_scoped(
        functools.partial(_body, x_hbm, ckv_hbm, wq_hbm, wuk_hbm, wuv_hbm, wo_hbm, w1_hbm,
                          b1_hbm, w2_hbm, o_hbm, out_sem, out_v, *scratch),
        pltpu.SemaphoreType.DMA((_n_copies(),)))
    pltpu.make_async_copy(out_v, o_hbm, out_sem).wait()


@jax.jit
def pallas_sequential_preLN__compressed_kv_cla__dense_activation_mish__decode_kernel(
    A_x: jax.Array,
    A_c_kv: jax.Array,
    A_w_q: jax.Array,
    A_w_uk: jax.Array,
    A_w_uv: jax.Array,
    A_w_o: jax.Array,
    B_x: jax.Array,
    B_w1: jax.Array,
    B_b1: jax.Array,
    B_w2: jax.Array,
):
    del B_x
    bf16 = jnp.bfloat16
    wq = A_w_q.reshape(_M * _H, _D)
    wuk = A_w_uk.reshape(_C * _H, _D)
    wuv = A_w_uv.reshape(_C * _H, _D)
    wo = A_w_o.reshape(_H * _D, _M)
    hbm = pl.BlockSpec(memory_space=pl.ANY)
    out = pl.pallas_call(
        _kernel,
        out_shape=jax.ShapeDtypeStruct((_B, _M), A_x.dtype),
        in_specs=[hbm] * 9,
        out_specs=hbm,
        scratch_shapes=[
            pltpu.SemaphoreType.DMA(()),
            pltpu.VMEM((_B, _M), bf16),
            pltpu.VMEM((_B, _M), bf16),
            pltpu.VMEM((_B, _SK, _C), bf16),
            pltpu.VMEM((_M * _H, _D), bf16),
            pltpu.VMEM((_C * _H, _D), bf16),
            pltpu.VMEM((_C * _H, _D), bf16),
            pltpu.VMEM((_H * _D, _M), bf16),
            pltpu.VMEM((_M, _F), bf16),
            pltpu.VMEM((_F,), bf16),
            pltpu.VMEM((_F, _M), bf16),
            pltpu.VMEM((4, 16, 2 * _C), bf16),
            pltpu.VMEM((4, 16, _D), jnp.float32),
            pltpu.VMEM((_B, _H, _C), jnp.float32),
            pltpu.VMEM((_B, _H, _C), jnp.float32),
        ],
        compiler_params=pltpu.CompilerParams(vmem_limit_bytes=60 * 1024 * 1024),
    )(A_x.reshape(_B, _M), A_c_kv, wq, wuk, wuv, wo, B_w1, B_b1, B_w2)
    return out.reshape(_B, 1, _M)
```

```python
import functools

import jax
import jax.numpy as jnp
import jax.experimental.pallas as pl
import jax.experimental.pallas.tpu as pltpu

_B = 2
_M = 512
_H = 32
_D = 128
_C = 512
_SK = 8192
_F = 1792

_KV_CH = 4096
_KV_SUB = 1024

_W2_MXU = (896, 512)
_W2_VPU = (224, 96, 48, 16)

_NT = (((1,), (1,)), ((), ()))


def _n_copies():
    return 7 + _B * (_SK // _KV_CH) + len(_W2_MXU) + len(_W2_VPU)


def _layernorm(v):
    m = jnp.mean(v, axis=-1, keepdims=True)
    c = v - m
    var = jnp.mean(c * c, axis=-1, keepdims=True)
    return c / jnp.sqrt(var + 1e-5)


def _pair_rows(w32_ref, g, jj, n):
    rows = w32_ref.shape[0]
    view = w32_ref.at[pl.ds(pl.multiple_of(4 * g, 4), rows - 12)]
    w = view[pl.ds(jj, n, stride=_H // 2), :]
    return pltpu.bitcast(w, jnp.bfloat16)


def _body(x_hbm, ckv_hbm, wq_hbm, wuk_hbm, wuv_hbm, wo_hbm, w1_hbm, b1_hbm, w2_hbm,
          o_hbm, out_v,
          x_v, ckv_v, wq_v, wuk_v, wuv_v, wo_v, w1_v, b1_v, w2_v,
          l_s, t_s, qa_s, cl_s, a_s, sems):
    f32, bf16 = jnp.float32, jnp.bfloat16

    n_kv = _SK // _KV_CH
    w2_blocks = _W2_MXU + _W2_VPU
    w2_off = [sum(w2_blocks[:i]) for i in range(len(w2_blocks))]
    copies = []

    def queue(src, dst):
        copies.append(pltpu.make_async_copy(src, dst, sems.at[len(copies)]))
        return copies[-1]

    cp_wq, cp_x, cp_b1 = queue(wq_hbm, wq_v), queue(x_hbm, x_v), queue(b1_hbm, b1_v)
    cp_wuk = queue(wuk_hbm, wuk_v)
    kv_sem0 = len(copies)
    for b in range(_B):
        for c in range(n_kv):
            sl = pl.ds(c * _KV_CH, _KV_CH)
            queue(ckv_hbm.at[b, sl], ckv_v.at[b, sl])
    cp_wuv, cp_wo, cp_w1 = queue(wuv_hbm, wuv_v), queue(wo_hbm, wo_v), queue(w1_hbm, w1_v)
    cp_w2 = [queue(w2_hbm.at[pl.ds(f0, n)], w2_v.at[pl.ds(f0, n)])
             for f0, n in zip(w2_off, w2_blocks)]
    assert len(copies) == _n_copies()
    for cp in copies:
        cp.start()

    ri = jax.lax.broadcasted_iota(jnp.int32, (128, 256), 0)
    ci = jax.lax.broadcasted_iota(jnp.int32, (128, 256), 1)
    dup = jnp.where(ri == (ci >> 1), 1.0, 0.0).astype(bf16)
    rt = jax.lax.broadcasted_iota(jnp.int32, (256, 128), 0)
    ct = jax.lax.broadcasted_iota(jnp.int32, (256, 128), 1)
    dup_t = jnp.where((rt >> 1) == ct, 1.0, 0.0).astype(bf16)

    row16 = jax.lax.broadcasted_iota(jnp.int32, (16, 2 * _C), 0)
    lane16 = jax.lax.broadcasted_iota(jnp.int32, (16, 2 * _C), 1)
    hh16 = row16 & 7
    par_ok = (lane16 & 1) == (hh16 & 1)

    def expand(v):
        return jnp.concatenate(
            [jnp.dot(v[:, 128 * t:128 * (t + 1)], dup, preferred_element_type=f32)
             for t in range(_C // 128)], axis=1)

    def store_pair_lhs(v2):
        for jj in range(4):
            keep = jnp.logical_and(par_ok, (hh16 >> 1) == jj)
            l_s[jj] = jnp.where(keep, v2, 0.0).astype(bf16)

    wq32 = wq_v.bitcast(jnp.uint32)
    wuk32 = wuk_v.bitcast(jnp.uint32)
    wuv32 = wuv_v.bitcast(jnp.uint32)

    cp_x.wait()
    x2 = x_v[...].astype(f32)
    xf = jnp.concatenate(
        [jnp.broadcast_to(x2[b:b + 1], (8, _M)) for b in range(_B)], axis=0)
    xn = _layernorm(xf).astype(bf16)
    store_pair_lhs(expand(xn))
    cp_wq.wait()

    scale = _D ** -0.5
    log2e = 1.4426950408889634

    def q_group(g, _):
        acc = jnp.zeros((16, _D), f32)
        for jj in range(4):
            acc = acc + jnp.dot(l_s[jj], _pair_rows(wq32, g, jj, _M),
                                preferred_element_type=f32)
        t_s[g] = acc
        return 0

    jax.lax.fori_loop(0, 4, q_group, 0)

    cp_wuk.wait()
    hh_q = jax.lax.broadcasted_iota(jnp.int32, (16, _D), 0) & 7

    def qa_group(g, _):
        q = t_s[g]
        acc = jnp.zeros((16, 2 * _C), f32)
        for jj in range(4):
            lq = jnp.where((hh_q >> 1) == jj, q, 0.0).astype(bf16)
            acc = acc + jax.lax.dot_general(lq, _pair_rows(wuk32, g, jj, _C), _NT,
                                            preferred_element_type=f32)
        tm = jnp.where(par_ok, acc * (scale * log2e), 0.0).astype(bf16)
        qa = jnp.concatenate(
            [jnp.dot(tm[:, 256 * t:256 * (t + 1)], dup_t, preferred_element_type=f32)
             for t in range(_C // 128)], axis=1)
        qa_s[0, pl.ds(pl.multiple_of(8 * g, 8), 8), :] = qa[0:8]
        qa_s[1, pl.ds(pl.multiple_of(8 * g, 8), 8), :] = qa[8:16]
        return 0

    jax.lax.fori_loop(0, 4, qa_group, 0)

    n_sub = _SK // _KV_SUB
    sub_per_dma = _KV_CH // _KV_SUB

    def kv_step(i, carry):
        m, l, acc = carry
        b = i // n_sub
        s_idx = i - b * n_sub
        off = pl.multiple_of(s_idx * _KV_SUB, _KV_SUB)

        @pl.when(s_idx % sub_per_dma == 0)
        def _():
            sl = pl.ds(pl.multiple_of((s_idx // sub_per_dma) * _KV_CH, _KV_CH), _KV_CH)
            pltpu.make_async_copy(ckv_hbm.at[b, sl], ckv_v.at[b, sl],
                                  sems.at[kv_sem0 + i // sub_per_dma]).wait()

        first = s_idx == 0
        m = jnp.where(first, -jnp.inf, m)
        l = jnp.where(first, 0.0, l)
        acc = jnp.where(first, 0.0, acc)
        qa = qa_s[b].astype(bf16)
        ck = ckv_v[b, pl.ds(off, _KV_SUB), :]
        s = jax.lax.dot_general(qa, ck, _NT, preferred_element_type=f32)
        m_new = jnp.maximum(m, jnp.max(s, axis=-1, keepdims=True))
        alpha = jnp.exp2(m - m_new)
        p = jnp.exp2(s - m_new)
        l = alpha * l + jnp.sum(p, axis=-1, keepdims=True)
        acc = alpha * acc + jnp.dot(p.astype(bf16), ck, preferred_element_type=f32)

        @pl.when(s_idx == n_sub - 1)
        def _():
            cl_s[b] = acc / l

        return m_new, l, acc

    jax.lax.fori_loop(
        0, _B * n_sub, kv_step,
        (jnp.zeros((_H, 1), f32), jnp.zeros((_H, 1), f32), jnp.zeros((_H, _C), f32)))

    cp_wuv.wait()

    def ctx_group(g, _):
        r0 = pl.multiple_of(8 * g, 8)
        cl = jnp.concatenate([cl_s[0, pl.ds(r0, 8), :], cl_s[1, pl.ds(r0, 8), :]], axis=0)
        cl2 = expand(cl.astype(bf16))
        acc = jnp.zeros((16, _D), f32)
        for jj in range(4):
            keep = jnp.logical_and(par_ok, (hh16 >> 1) == jj)
            lhs = jnp.where(keep, cl2, 0.0).astype(bf16)
            acc = acc + jnp.dot(lhs, _pair_rows(wuv32, g, jj, _C),
                                preferred_element_type=f32)
        t_s[g] = acc
        return 0

    jax.lax.fori_loop(0, 4, ctx_group, 0)

    cp_wo.wait()

    def out_group(g, acc):
        ctx = t_s[g]
        lhs = jnp.concatenate(
            [jnp.where(hh_q == k, ctx, 0.0).astype(bf16) for k in range(8)], axis=1)
        w = wo_v[pl.ds(pl.multiple_of(g * 8 * _D, 8 * _D), 8 * _D), :]
        return acc + jnp.dot(lhs, w, preferred_element_type=f32)

    part = jax.lax.fori_loop(0, 4, out_group, jnp.zeros((16, _M), f32))
    attn = jnp.concatenate(
        [jnp.broadcast_to(jnp.sum(part[8 * b:8 * (b + 1)], axis=0, keepdims=True), (8, _M))
         for b in range(_B)], axis=0)
    h = xf + attn

    hn = _layernorm(h).astype(bf16)
    cp_b1.wait()
    cp_w1.wait()
    u = jnp.dot(hn, w1_v[...], preferred_element_type=f32)
    u = u + b1_v[...].astype(f32)[None, :]
    sp = jnp.log1p(jnp.exp(-jnp.abs(u))) + jnp.maximum(u, 0.0)
    act = (u * jnp.tanh(sp)).astype(bf16)

    f_vpu = sum(_W2_MXU)
    eye = ri[:, 0:128] == ci[:, 0:128]
    ones = jnp.ones((128, 128), bf16)
    for b in range(_B):
        for t in range(sum(_W2_VPU) // 128):
            c0 = f_vpu + 128 * t
            diag = jnp.where(eye, jnp.broadcast_to(act[8 * b:8 * b + 1, c0:c0 + 128], (128, 128)), 0)
            a_s[b, pl.ds(128 * t, 128), :] = jnp.dot(diag, ones, preferred_element_type=f32)

    y = h
    vacc = [jnp.zeros((8, _M), f32) for _ in range(_B)]
    for cp, f0, n in zip(cp_w2, w2_off, w2_blocks):
        cp.wait()
        if f0 < f_vpu:
            y = y + jnp.dot(act[:, f0:f0 + n], w2_v[pl.ds(f0, n), :], preferred_element_type=f32)
        else:
            for r in range(f0, f0 + n, 8):
                w = w2_v[pl.ds(r, 8), :].astype(f32)
                for b in range(_B):
                    a = a_s[b, pl.ds(r - f_vpu, 8), :]
                    vacc[b] = vacc[b] + w * jnp.concatenate([a] * (_M // 128), axis=1)
    y0 = y[0:8] + jnp.sum(vacc[0], axis=0, keepdims=True)
    y1 = y[8:16] + jnp.sum(vacc[1], axis=0, keepdims=True)

    sub = jax.lax.broadcasted_iota(jnp.int32, (8, _M), 0)
    out_v[...] = jnp.where(sub == 0, y0, y1)[0:_B].astype(bf16)
    cp_out = pltpu.make_async_copy(out_v, o_hbm, sems.at[_n_copies()])
    cp_out.start()
    cp_out.wait()


def _kernel(*refs):
    pl.run_scoped(functools.partial(_body, *refs), pltpu.SemaphoreType.DMA((_n_copies() + 1,)))


@jax.jit
def pallas_sequential_preLN__compressed_kv_cla__dense_activation_mish__decode_kernel(
    A_x: jax.Array,
    A_c_kv: jax.Array,
    A_w_q: jax.Array,
    A_w_uk: jax.Array,
    A_w_uv: jax.Array,
    A_w_o: jax.Array,
    B_x: jax.Array,
    B_w1: jax.Array,
    B_b1: jax.Array,
    B_w2: jax.Array,
):
    del B_x
    bf16 = jnp.bfloat16
    wq = A_w_q.reshape(_M * _H, _D)
    wuk = A_w_uk.reshape(_C * _H, _D)
    wuv = A_w_uv.reshape(_C * _H, _D)
    wo = A_w_o.reshape(_H * _D, _M)
    hbm = pl.BlockSpec(memory_space=pl.ANY)
    out = pl.pallas_call(
        _kernel,
        out_shape=jax.ShapeDtypeStruct((_B, _M), A_x.dtype),
        in_specs=[hbm] * 9,
        out_specs=hbm,
        scratch_shapes=[
            pltpu.VMEM((_B, _M), bf16),
            pltpu.VMEM((_B, _M), bf16),
            pltpu.VMEM((_B, _SK, _C), bf16),
            pltpu.VMEM((_M * _H, _D), bf16),
            pltpu.VMEM((_C * _H, _D), bf16),
            pltpu.VMEM((_C * _H, _D), bf16),
            pltpu.VMEM((_H * _D, _M), bf16),
            pltpu.VMEM((_M, _F), bf16),
            pltpu.VMEM((_F,), bf16),
            pltpu.VMEM((_F, _M), bf16),
            pltpu.VMEM((4, 16, 2 * _C), bf16),
            pltpu.VMEM((4, 16, _D), jnp.float32),
            pltpu.VMEM((_B, _H, _C), jnp.float32),
            pltpu.VMEM((_B, _H, _C), jnp.float32),
            pltpu.VMEM((_B, sum(_W2_VPU), 128), jnp.float32),
        ],
        compiler_params=pltpu.CompilerParams(vmem_limit_bytes=60 * 1024 * 1024),
    )(A_x.reshape(_B, _M), A_c_kv, wq, wuk, wuv, wo, B_w1, B_b1, B_w2)
    return out.reshape(_B, 1, _M)
```
